```python
import jax
import jax.numpy as jnp

def _softmax(x, axis=-1):
    return jax.nn.softmax(x, axis=axis)
def _gelu(x):
    return jax.nn.gelu(x, approximate=True)
def _silu(x):
    return jax.nn.silu(x)
def _sigmoid(x):
    return jax.nn.sigmoid(x)
def _layernorm(x, axis=-1, eps=1e-5):
    m = jnp.mean(x, axis=axis, keepdims=True)
    v = jnp.var(x, axis=axis, keepdims=True)
    return (x - m) / jnp.sqrt(v + eps)
def _scatter_add(tgt, idx, src, axis=0):
    return tgt.at[idx].add(src)
def _segment_sum(src, seg, n):
    return jax.ops.segment_sum(src, seg, n)
class _Rng:
    def __init__(self, key):
        self._k = key
    def _next(self):
        self._k, sub = jax.random.split(self._k)
        return sub
    def normal(self, shape):
        return jax.random.normal(self._next(), shape, dtype=jnp.bfloat16)
    def randint(self, lo, hi, shape):
        return jax.random.randint(self._next(), shape, lo, hi, dtype=jnp.int32)
    def uniform(self, shape, lo=0.0, hi=1.0):
        return jax.random.uniform(self._next(), shape, jnp.bfloat16, lo, hi)
    def permutation(self, n):
        return jax.random.permutation(self._next(), n)


kernel_name = 'sequential_preLN__sliding_block__glu_gated_glu__prompt'

def _fwd_setup_inputs():
    _rng = _Rng(jax.random.key(int.from_bytes(__import__("os").urandom(4), "little")))
    _w = (lambda a: (lambda t: t.astype(jnp.bfloat16) if jnp.issubdtype(t.dtype, jnp.floating) else t)(jnp.asarray(a)))
    def _A_setup():
        B, S, D = 1, 2048, 512
        return {
            "x": _w((lambda *s: _rng.normal(s) * 0.05)(B, S, D)),
            "wqkv": _w((lambda *s: _rng.normal(s) * 0.05)(D, 3 * D)),
            "wo": _w((lambda *s: _rng.normal(s) * 0.05)(D, D)),
        }
    _A_in = _A_setup()

    def _B_setup():
        B, S, D, F = 1, 2048, 512, 1376
        return {
            "x": _w((lambda *s: _rng.normal(s) * 0.05)(B, S, D)),
            "w_gate": _w((lambda *s: _rng.normal(s) * 0.05)(D, F)),
            "w_up": _w((lambda *s: _rng.normal(s) * 0.05)(D, F)),
            "w_down": _w((lambda *s: _rng.normal(s) * 0.05)(F, D)),
        }
    _B_in = _B_setup()

    return {
        "A_x": _A_in["x"],
        "A_wqkv": _A_in["wqkv"],
        "A_wo": _A_in["wo"],
        "B_x": _B_in["x"],
        "B_w_gate": _B_in["w_gate"],
        "B_w_up": _B_in["w_up"],
        "B_w_down": _B_in["w_down"],
    }

def _fwd_reference(A_x, A_wqkv, A_wo, B_x, B_w_gate, B_w_up, B_w_down):
    def _A_ref(x, wqkv, wo):
        B, S, D = x.shape
        H = 32; Dh = D // H; W = 256
        qkv = (lambda x, *d: x.transpose(*d))((x @ wqkv).reshape(B, S, 3, H, Dh), 2, 0, 3, 1, 4)
        q, k, v = qkv[0], qkv[1], qkv[2]
        scores = jnp.einsum("bhqd,bhkd->bhqk", q, k) * (Dh ** -0.5)
        idx = jnp.arange(S)
        mask = (idx[:, None] - idx[None, :] >= 0) & (idx[:, None] - idx[None, :] < W)
        scores = jnp.where(mask[None, None], scores, -1e9)
        p = _softmax(scores, axis=-1)
        o = jnp.einsum("bhqk,bhkd->bhqd", p, v)
        return (lambda x, *d: x.transpose(*d))(o, 0, 2, 1, 3).reshape(B, S, D) @ wo

    def _B_ref(x, w_gate, w_up, w_down):
        g = jnp.einsum("bsd,df->bsf", x, w_gate)
        u = jnp.einsum("bsd,df->bsf", x, w_up)
        h = _sigmoid(g) * u
        return jnp.einsum("bsf,fd->bsd", h, w_down)

    x = A_x
    h = x + _A_ref(_layernorm(x, axis=-1), A_wqkv, A_wo)
    h2 = h + _B_ref(_layernorm(h, axis=-1), B_w_gate, B_w_up, B_w_down)
    return h2


def setup_inputs():
    _inp = _fwd_setup_inputs()
    _gk = jax.random.fold_in(jax.random.key(int.from_bytes(__import__("os").urandom(4), "little")), 2**31 - 1)
    _shapes = [[1, 2048, 512]]
    _dtypes = ['bfloat16']
    _gks = jax.random.split(_gk, len(_shapes))
    _gs = [jax.random.normal(k, s, dtype=jnp.dtype(d)) * 0.05 for k, s, d in zip(_gks, _shapes, _dtypes)]
    _inp["grad_out"] = _gs[0]
    return _inp

def reference(A_x, A_wqkv, A_wo, B_w_gate, B_w_up, B_w_down, B_x, grad_out):
    _const = dict(B_x=B_x)
    def _f(*_d):
        return _fwd_reference(**{'A_x': _d[0], 'A_wqkv': _d[1], 'A_wo': _d[2], 'B_w_gate': _d[3], 'B_w_up': _d[4], 'B_w_down': _d[5], **_const})
    _out, _vjp = jax.vjp(_f, A_x, A_wqkv, A_wo, B_w_gate, B_w_up, B_w_down)
    _grads = _vjp(grad_out)
    _out0 = jnp.asarray(_out)
    return (_out0, *[jnp.asarray(_g) for _g in _grads])
```

```python
import jax
import jax.numpy as jnp
from jax import lax
import jax.experimental.pallas as pl
import jax.experimental.pallas.tpu as pltpu

S, D, F = 2048, 512, 1376
W = 256
R = 256
NB = R // 128
TK = 288
BF, F32 = jnp.bfloat16, jnp.float32
NN = (((1,), (0,)), ((), ()))
NT = (((1,), (1,)), ((), ()))
TN = (((0,), (0,)), ((), ()))


def _dot(a, b, dims=NN):
    return lax.dot_general(a, b, dims, preferred_element_type=F32)


def _ln(x):
    m = jnp.mean(x, axis=-1, keepdims=True)
    c = x - m
    r = lax.rsqrt(jnp.mean(c * c, axis=-1, keepdims=True) + 1e-5)
    return c * r, r


def _ln_bwd(dy, y, r):
    return r * (dy - jnp.mean(dy, axis=-1, keepdims=True)
                - y * jnp.mean(dy * y, axis=-1, keepdims=True))


def _blockdiag(blk):
    hd = lax.broadcasted_iota(jnp.int32, (16, 128), 1) // 16
    blk = pltpu.bitcast(blk, jnp.int32)
    z = jnp.zeros_like(blk)
    return [pltpu.bitcast(jnp.concatenate(
        [jnp.where(hd == 4 * s + h, blk, z) for h in range(4)], axis=0), BF)
            for s in range(2)]


def _gather_heads(mt, pts, t):
    rs = []
    for s in range(2):
        parts = [pts[s]]
        if t > 0:
            parts = [jnp.zeros((32 * t, 128), BF)] + parts
        if t < 3:
            parts = parts + [jnp.zeros((96 - 32 * t, 128), BF)]
        rs.append(_dot(mt[64 * s:64 * s + 64], jnp.concatenate(parts, axis=0)))
    h4 = (lax.broadcasted_iota(jnp.int32, (32, 128), 1) // 16) % 4
    tt = jnp.concatenate(rs, axis=0).T
    o = tt[0:32]
    for h in range(1, 4):
        o = jnp.where(h4 == h, tt[32 * h:32 * h + 32], o)
    return o


def _kernel(x_ref, wqkv_ref, wo_h, wg_h, wu_h, wd_h, go_h,
            out_h, dx_ref, dwqkv_ref, dwo_h, dwg_h, dwu_h, dwd_h,
            wo_ref, wg_ref, wu_ref, wd_ref, go_ref, out_ref, dwo_ref, dwg_ref, dwu_ref, dwd_ref, sems,
            xn_s, q_s, k_s, v_s, kt_s, vt_s, p_s, o_s, do_s, dq_s, dk_s, dv_s, dh_s,
            aqkv, ao, ag, au, ad):
    cp = pltpu.make_async_copy
    ins = [cp(a, b, sems.at[n]) for n, (a, b) in enumerate(
        [(wo_h, wo_ref), (wg_h, wg_ref), (wu_h, wu_ref), (wd_h, wd_ref), (go_h, go_ref)])]
    for d_ in ins:
        d_.start()
    for g in range(4):
        k_s[g, 0:W] = jnp.zeros((W, 128), BF)
        v_s[g, 0:W] = jnp.zeros((W, 128), BF)
        for b in range(2):
            kt_s[g, b] = jnp.zeros((128, 128), BF)
            vt_s[g, b] = jnp.zeros((128, 128), BF)
    dk_s[...] = jnp.zeros(dk_s.shape, F32)
    dv_s[...] = jnp.zeros(dv_s.shape, F32)
    for a in (aqkv, ao, ag, au, ad):
        a[...] = jnp.zeros(a.shape, F32)

    def proj(c, _):
        r0 = pl.multiple_of(c * R, R)
        y, _r = _ln(x_ref[pl.ds(r0, R)].astype(F32))
        yb = y.astype(BF)
        xn_s[pl.ds(r0, R)] = yb
        qkv = _dot(yb, wqkv_ref[...])
        for g in range(4):
            q_s[g, pl.ds(r0, R)] = (qkv[:, 128 * g:128 * g + 128] * 0.25).astype(BF)
            k = qkv[:, D + 128 * g:D + 128 * g + 128]
            v = qkv[:, 2 * D + 128 * g:2 * D + 128 * g + 128]
            k_s[g, pl.ds(r0 + W, R)] = k.astype(BF)
            v_s[g, pl.ds(r0 + W, R)] = v.astype(BF)
            for b in range(NB):
                kt_s[g, c * NB + 2 + b] = k[128 * b:128 * b + 128].T.astype(BF)
                vt_s[g, c * NB + 2 + b] = v[128 * b:128 * b + 128].T.astype(BF)
        return 0
    lax.fori_loop(0, S // R, proj, 0)

    def window(ref, g, blk):
        return jnp.concatenate([ref[g, blk + j] for j in range(3)], axis=1)

    def fwd_a(c, i, t):
        g, b = i // NB, i % NB
        qt = pl.multiple_of(c * R + b * 128 + 32 * t, 32)
        qbd = jnp.concatenate(_blockdiag(q_s[g, pl.ds(qt, 32)]), axis=0)
        return qt, _dot(k_s[g, pl.ds(qt, TK)], qbd, NT)

    def fwd_b(c, i, t, qt, sc2, vw, edge):
        g, b = i // NB, i % NB
        jj = lax.broadcasted_iota(jnp.int32, (32, 128), 0)
        ii = lax.broadcasted_iota(jnp.int32, (32, 128), 1) % 32
        low = jj <= ii
        row = []
        for s in range(2):
            sc = sc2[:, 128 * s:128 * s + 128]
            first = jnp.where(qt >= W, sc[0:32], -1e9) if edge else sc[0:32]
            grp = [jnp.where(low, sc[256:288], first)]
            for j in range(1, 8):
                grp.append(jnp.where(qt + 32 * j >= W, sc[32 * j:32 * j + 32], -1e9)
                           if edge else sc[32 * j:32 * j + 32])
            z = jnp.concatenate(grp, axis=0)
            e = jnp.exp(z - jnp.max(z, axis=0, keepdims=True))
            p = e * (1.0 / jnp.sum(e, axis=0, keepdims=True))
            pt = jnp.concatenate([jnp.where(low, 0.0, p[0:32]), p[32:256],
                                  jnp.where(low, p[0:32], 0.0)], axis=0).astype(BF)
            p_s[c % 2, i, 2 * t + s] = pt
            row.append(pt)
        o_s[c % 2, g, pl.ds(pl.multiple_of(b * 128 + 32 * t, 32), 32)] = (
            _gather_heads(vw, row, t).astype(BF))

    def bwd_a(c, i, t):
        g, b = i // NB, i % NB
        qt = pl.multiple_of(c * R + b * 128 + 32 * t, 32)
        dbd = jnp.concatenate(
            _blockdiag(do_s[g, pl.ds(pl.multiple_of(b * 128 + 32 * t, 32), 32)]), axis=0)
        dp2 = _dot(v_s[g, pl.ds(qt, TK)], dbd, NT)
        ps = [p_s[c % 2, i, 2 * t + s] for s in range(2)]
        dv_s[g, pl.ds(qt, TK)] += _dot(jnp.concatenate(ps, axis=1), dbd)
        return qt, dp2, ps

    def bwd_b(c, i, t, qt, dp2, ps, kw):
        g = i // NB
        qbd = jnp.concatenate(_blockdiag(q_s[g, pl.ds(qt, 32)]), axis=0)
        row = []
        for s in range(2):
            p = ps[s].astype(F32)
            pd = p * dp2[:, 128 * s:128 * s + 128]
            row.append((pd - p * jnp.sum(pd, axis=0, keepdims=True)).astype(BF))
        dk_s[g, pl.ds(qt, TK)] += _dot(jnp.concatenate(row, axis=1), qbd)
        dq_s[g, pl.ds(qt, 32)] = (_gather_heads(kw, row, t) * 0.25).astype(BF)

    def fwd_only(i, _):
        vw = window(vt_s, i // NB, i % NB)
        a = fwd_a(0, i, 0)
        for t in range(4):
            nxt = fwd_a(0, i, t + 1) if t < 3 else None
            fwd_b(0, i, t, *a, vw, True)
            a = nxt
        return 0
    lax.fori_loop(0, 4 * NB, fwd_only, 0)

    for d_ in ins:
        d_.wait()

    def chunk(c, _):
        r0 = pl.multiple_of(c * R, R)
        cn = jnp.where(c + 1 < S // R, c + 1, c - 1)

        o = jnp.concatenate([o_s[c % 2, g] for g in range(4)], axis=1)
        h = x_ref[pl.ds(r0, R)].astype(F32) + _dot(o, wo_ref[...])
        hn, rstd = _ln(h)
        hb = hn.astype(BF)
        go = go_ref[pl.ds(r0, R)]
        sg = jax.nn.sigmoid(_dot(hb, wg_ref[...], NT))
        u = _dot(hb, wu_ref[...], NT)
        act = sg * u
        actb = act.astype(BF)
        out_ref[pl.ds(r0, R)] = (h + _dot(actb, wd_ref[...])).astype(BF)
        ad[...] += _dot(actb, go, TN)
        da = _dot(go, wd_ref[...], NT)
        dub = (da * sg).astype(BF)
        dgb = (da * act * (1.0 - sg)).astype(BF)
        ag[...] += _dot(dgb, hb, TN)
        au[...] += _dot(dub, hb, TN)
        dhn = _dot(dgb, wg_ref[...]) + _dot(dub, wu_ref[...])
        dh = go.astype(F32) + _ln_bwd(dhn, hn, rstd)
        dh_s[pl.ds(r0, R)] = dh
        dhb = dh.astype(BF)
        ao[...] += _dot(o, dhb, TN)
        do = _dot(dhb, wo_ref[...], NT).astype(BF)
        for g in range(4):
            do_s[g] = do[:, 128 * g:128 * g + 128]

        def att_bwd(i, _):
            g, b = i // NB, i % NB
            kw = window(kt_s, g, c * NB + b)
            vw = window(vt_s, g, cn * NB + b)
            fa = fwd_a(cn, i, 0)
            for t in range(4):
                ba = bwd_a(c, i, t)
                fwd_b(cn, i, t, *fa, vw, False)
                if t < 3:
                    fa = fwd_a(cn, i, t + 1)
                bwd_b(c, i, t, *ba, kw)
            return 0
        lax.fori_loop(0, 4, lambda g, _: att_bwd(g * NB + 1, att_bwd(g * NB, 0)), 0)
        return 0
    lax.fori_loop(0, S // R, chunk, 0)

    dwo_ref[...] = ao[...].astype(BF)
    dwg_ref[...] = ag[...].astype(BF)
    dwu_ref[...] = au[...].astype(BF)
    dwd_ref[...] = ad[...].astype(BF)
    outs = [cp(a, b, sems.at[n]) for n, (a, b) in enumerate(
        [(dwo_ref, dwo_h), (dwg_ref, dwg_h), (dwu_ref, dwu_h), (dwd_ref, dwd_h), (out_ref, out_h)])]
    for d_ in outs:
        d_.start()

    def proj_bwd(c, _):
        r0 = pl.multiple_of(c * R, R)
        d = jnp.concatenate(
            [dq_s[g, pl.ds(r0, R)] for g in range(4)]
            + [dk_s[g, pl.ds(r0 + W, R)].astype(BF) for g in range(4)]
            + [dv_s[g, pl.ds(r0 + W, R)].astype(BF) for g in range(4)], axis=1)
        aqkv[...] += _dot(xn_s[pl.ds(r0, R)], d, TN)
        dxn = _dot(d, wqkv_ref[...], NT)
        y, r = _ln(x_ref[pl.ds(r0, R)].astype(F32))
        dx_ref[pl.ds(r0, R)] = (dh_s[pl.ds(r0, R)] + _ln_bwd(dxn, y, r)).astype(BF)
        return 0
    lax.fori_loop(0, S // R, proj_bwd, 0)
    dwqkv_ref[...] = aqkv[...].astype(BF)
    for d_ in outs:
        d_.wait()


@jax.jit
def pallas_sequential_preLN__sliding_block__glu_gated_glu__prompt_kernel(
    A_x, A_wqkv, A_wo, B_x, B_w_gate, B_w_up, B_w_down, grad_out):
    sd = jax.ShapeDtypeStruct
    vm = pltpu.VMEM
    hb = pl.BlockSpec(memory_space=pl.ANY)
    outs = pl.pallas_call(
        _kernel,
        out_shape=[sd((S, D), BF), sd((S, D), BF), sd((D, 3 * D), BF), sd((D, D), BF),
                   sd((F, D), BF), sd((F, D), BF), sd((F, D), BF)],
        in_specs=[pl.BlockSpec(memory_space=vm)] * 2 + [hb] * 5,
        out_specs=[hb] + [pl.BlockSpec(memory_space=vm)] * 2 + [hb] * 4,
        scratch_shapes=[
            vm((D, D), BF), vm((F, D), BF), vm((F, D), BF), vm((F, D), BF), vm((S, D), BF),
            vm((S, D), BF), vm((D, D), BF), vm((F, D), BF), vm((F, D), BF), vm((F, D), BF),
            pltpu.SemaphoreType.DMA((5,)),
            vm((S, D), BF), vm((4, S, 128), BF), vm((4, S + W, 128), BF), vm((4, S + W, 128), BF),
            vm((4, S // 128 + 2, 128, 128), BF), vm((4, S // 128 + 2, 128, 128), BF),
            vm((2, 4 * NB, 8, TK, 128), BF), vm((2, 4, R, 128), BF), vm((4, R, 128), BF),
            vm((4, S, 128), BF), vm((4, S + W, 128), F32), vm((4, S + W, 128), F32),
            vm((S, D), F32),
            vm((D, 3 * D), F32), vm((D, D), F32), vm((F, D), F32), vm((F, D), F32), vm((F, D), F32),
        ],
        compiler_params=pltpu.CompilerParams(vmem_limit_bytes=110 * 1024 * 1024),
    )(A_x.reshape(S, D), A_wqkv, A_wo, B_w_gate.T, B_w_up.T, B_w_down, grad_out.reshape(S, D))
    return (outs[0].reshape(1, S, D), outs[1].reshape(1, S, D), outs[2], outs[3],
            outs[4].T, outs[5].T, outs[6])
```
